```python
import os as _os
_os.environ.setdefault("JAX_PLATFORMS", "cpu")
import jax
import jax.numpy as jnp

def _softmax(x, axis=-1):
    return jax.nn.softmax(x, axis=axis)
def _gelu(x):
    return jax.nn.gelu(x, approximate=True)
def _silu(x):
    return jax.nn.silu(x)
def _sigmoid(x):
    return jax.nn.sigmoid(x)
def _layernorm(x, axis=-1, eps=1e-5):
    m = jnp.mean(x, axis=axis, keepdims=True)
    v = jnp.var(x, axis=axis, keepdims=True)
    return (x - m) / jnp.sqrt(v + eps)
def _scatter_add(tgt, idx, src, axis=0):
    return tgt.at[idx].add(src)
def _segment_sum(src, seg, n):
    return jax.ops.segment_sum(src, seg, n)
class _Rng:
    def __init__(self, key):
        self._k = key
    def _next(self):
        self._k, sub = jax.random.split(self._k)
        return sub
    def normal(self, shape):
        return jax.random.normal(self._next(), shape, dtype=jnp.bfloat16)
    def randint(self, lo, hi, shape):
        return jax.random.randint(self._next(), shape, lo, hi, dtype=jnp.int32)
    def uniform(self, shape, lo=0.0, hi=1.0):
        return jax.random.uniform(self._next(), shape, jnp.bfloat16, lo, hi)
    def permutation(self, n):
        return jax.random.permutation(self._next(), n)


kernel_name = 'sequential_preLN__sliding_local_dilated__dense_activation_relu__prompt'

def setup_inputs():
    _rng = _Rng(jax.random.key(int.from_bytes(__import__("os").urandom(4), "little")))
    _w = (lambda a: (lambda t: t.astype(jnp.bfloat16) if jnp.issubdtype(t.dtype, jnp.floating) else t)(jnp.asarray(a)))
    def _A_setup():
        B, S, D = 1, 2048, 1024
        return {
            "x": _w((lambda *s: _rng.normal(s) * 0.05)(B, S, D)),
            "wqkv": _w((lambda *s: _rng.normal(s) * 0.05)(D, 3 * D)),
            "wo": _w((lambda *s: _rng.normal(s) * 0.05)(D, D)),
        }
    _A_in = _A_setup()

    def _B_setup():
        B, S, D, Dff = 1, 2048, 1024, 3584
        return {
            "x": _w((lambda *s: _rng.normal(s) * 0.05)(B, S, D)),
            "w1": _w((lambda *s: _rng.normal(s) * 0.05)(D, Dff)),
            "w2": _w((lambda *s: _rng.normal(s) * 0.05)(Dff, D)),
        }
    _B_in = _B_setup()

    return {
        "A_x": _A_in["x"],
        "A_wqkv": _A_in["wqkv"],
        "A_wo": _A_in["wo"],
        "B_x": _B_in["x"],
        "B_w1": _B_in["w1"],
        "B_w2": _B_in["w2"],
    }

def reference(A_x, A_wqkv, A_wo, B_x, B_w1, B_w2):
    def _A_ref(x, wqkv, wo):
        B, S, D = x.shape
        H = 32; Dh = D // H
        W, dil = 8, 2
        qkv = (lambda x, *d: x.transpose(*d))((x @ wqkv).reshape(B, S, 3, H, Dh), 2, 0, 3, 1, 4)
        q, k, v = qkv[0], qkv[1], qkv[2]
        scale = Dh ** -0.5
        pos = jnp.arange(S)
        off = jnp.arange(W) * dil
        idx = pos[:, None] - off[None, :]
        mask = idx >= 0
        idx_c = jnp.where(mask, idx, 0).reshape(-1)
        kg = k[:, :, idx_c, :].reshape(B, H, S, W, Dh)
        vg = v[:, :, idx_c, :].reshape(B, H, S, W, Dh)
        logits = jnp.einsum("bhsd,bhswd->bhsw", q, kg) * scale
        logits = jnp.where(mask[None, None, :, :], logits, -1e9)
        attn = _softmax(logits, axis=-1)
        o = jnp.einsum("bhsw,bhswd->bhsd", attn, vg)
        return (lambda x, *d: x.transpose(*d))(o, 0, 2, 1, 3).reshape(B, S, D) @ wo

    def _B_ref(x, w1, w2):
        h = jnp.einsum("bsd,df->bsf", x, w1)
        zero = jnp.zeros_like(h)
        h = jnp.maximum(h, zero)
        return jnp.einsum("bsf,fd->bsd", h, w2)

    x = A_x
    h = x + _A_ref(_layernorm(x, axis=-1), A_wqkv, A_wo)
    h2 = h + _B_ref(_layernorm(h, axis=-1), B_w1, B_w2)
    return h2
```

```python
import functools, contextlib
import jax, jax.numpy as jnp, numpy as np
from jax import lax
from jax.experimental import pallas as pl
from jax.experimental.pallas import tpu as pltpu

S, D, F, H, DH, W, DIL = 2048, 1024, 3584, 32, 32, 8, 2
HALO = 16
LOG2E = 1.4426950408889634
NT = D // 128
f32, bf16, i32 = jnp.float32, jnp.bfloat16, jnp.int32

def _ln(xf):
    m = jnp.mean(xf, axis=-1, keepdims=True)
    c = xf - m
    v = jnp.mean(c * c, axis=-1, keepdims=True)
    return c * lax.rsqrt(v + 1e-5)

def _lane_xor(x, bit):
    idx = lax.broadcasted_iota(i32, x.shape, 1) ^ bit
    return jnp.take_along_axis(x, idx, axis=1)

def _swap_tile_lane(tiles, tb, lb):
    lane = lax.broadcasted_iota(i32, tiles[0].shape, 1)
    hi = (lane & lb) != 0
    out = list(tiles)
    for t in range(len(tiles)):
        if t & tb:
            continue
        a, b = tiles[t], tiles[t | tb]
        c = jnp.where(hi, a, b)
        s = _lane_xor(c, lb)
        out[t] = jnp.where(hi, s, a)
        out[t | tb] = jnp.where(hi, b, s)
    return out

def _permute_cols(src_ref, dst_ref, c0, pr0, npr, chunk=16):
    for r0 in range(pr0, pr0 + npr, chunk):
        tiles = [src_ref[pl.ds(r0, chunk), pl.ds(c0 + t * 128, 128)] for t in range(NT)]
        for tb, lb in ((4, 16), (2, 8), (1, 4)):
            tiles = _swap_tile_lane(tiles, tb, lb)
        for t in range(NT):
            dst_ref[pl.ds(r0, chunk), pl.ds(c0 + t * 128, 128)] = tiles[t]

def _permute_rows(src_ref, dst_ref):
    def src_vreg(h4, h3, h2, a, d4):
        return (h4 << 5) | (h3 << 4) | (h2 << 3) | (a << 1) | d4
    def dst_vreg(d4, d3, d2, a, h4):
        return (d4 << 5) | (d3 << 4) | (d2 << 3) | (a << 1) | h4
    CW = 512
    sub = lax.broadcasted_iota(i32, (8, CW), 0)
    m4 = (sub & 4) != 0
    m2 = (sub & 2) != 0
    for a in range(4):
        for h4 in range(2):
            for d4 in range(2):
                for c0 in range(0, D, CW):
                    v = {}
                    for h3 in range(2):
                        for h2 in range(2):
                            r0 = src_vreg(h4, h3, h2, a, d4) * 8
                            v[h3, h2] = src_ref[pl.ds(r0, 8), pl.ds(c0, CW)]
                    for h2 in range(2):
                        A, B = v[0, h2], v[1, h2]
                        c = jnp.where(m4, A, B)
                        s = pltpu.roll(c, 4, 0)
                        v[0, h2] = jnp.where(m4, s, A)
                        v[1, h2] = jnp.where(m4, B, s)
                    for h3 in range(2):
                        A, B = v[h3, 0], v[h3, 1]
                        v[h3, 0] = jnp.where(m2, pltpu.roll(B, 2, 0), A)
                        v[h3, 1] = jnp.where(m2, B, pltpu.roll(A, 6, 0))
                    for d3 in range(2):
                        for d2 in range(2):
                            r0 = dst_vreg(d4, d3, d2, a, h4) * 8
                            dst_ref[pl.ds(r0, 8), pl.ds(c0, CW)] = v[d3, d2]

def _mo(x, m):
    return x if isinstance(x, int) else pl.multiple_of(x, m)

def _split(n, parts):
    b = [(n * j) // parts for j in range(parts + 1)]
    return [range(b[j], b[j + 1]) for j in range(parts)]

def make(TM=256, TB=256, R=16, FC=512, LNR=16, NCH=12, NWO=4, KP=4, flags=None, scopes=False,
         wo_at=4, ln1_pos="wo", ln2_pos="wo", unrollA=1, grp=True, PCH=128, wo_wait_at=4, x2_wait_at=9, T0=128):
    NA = S // TM
    NB = (S - T0) // TB
    TL = S - T0 - NB * TB
    CQ = 3 * D // NCH
    CW_ = D // NWO
    PM = TM // 2
    KC = D // KP
    scope = (lambda n: jax.named_scope(n)) if scopes else (lambda n: contextlib.nullcontext())

    def kernel(x_hbm, wqkv_hbm, wo_hbm, w1_hbm, w2_hbm, out_hbm,
               x_s, wqkv_s, wqkv_p, wo_s, wo_p, w1_s, w2_s,
               ln1_s, qkv_s, o_s, h_s, ln2_s, out_s,
               in_sem, out_sem):
        xb = x_hbm.bitcast(i32); wqb = wqkv_hbm.bitcast(i32); wob = wo_hbm.bitcast(i32)
        w1b = w1_hbm.bitcast(i32); w2b = w2_hbm.bitcast(i32); ob = out_hbm.bitcast(i32)
        sem_i = iter(range(100))
        def cp(src, dst):
            return pltpu.make_async_copy(src, dst, in_sem.at[next(sem_i)])
        cp_x0 = cp(xb.at[pl.ds(0, PM), :], x_s.at[pl.ds(0, PM), :])
        cp_w = [[cp(wqb.at[pl.ds(j * KC // 2, KC // 2), pl.ds(c * D, D)], wqkv_s.at[pl.ds(j * KC // 2, KC // 2), pl.ds(c * D, D)])
                 for j in range(KP)] for c in range(3)]
        cp_x1 = cp(xb.at[pl.ds(PM, PM), :], x_s.at[pl.ds(PM, PM), :])
        cp_x2 = cp(xb.at[pl.ds(2 * PM, S // 2 - 2 * PM), :], x_s.at[pl.ds(2 * PM, S // 2 - 2 * PM), :])
        cp_wo = cp(wob, wo_s)
        cp_w1 = cp(w1b, w1_s)
        cp_w2 = cp(w2b, w2_s)

        def ldb(ref, prow, nrows, cols=None):
            v = ref[pl.ds(prow, nrows // 2), :] if cols is None else ref[pl.ds(prow, nrows // 2), pl.ds(cols[0], cols[1])]
            return pltpu.bitcast(v, bf16)

        def ln1_rows(i, r, n):
            pr = _mo(i * PM + r // 2, 8)
            xf = ldb(x_s, pr, n).astype(f32)
            ln1_s[pl.ds(pr, n // 2), :] = pltpu.bitcast(_ln(xf).astype(bf16), i32)

        def ln2_rows(i, r, n):
            r0 = _mo((i + 1) * TM + r, 8)
            pr = _mo((i + 1) * PM + r // 2, 8)
            hf = h_s[pl.ds(r0, n), :]
            ln2_s[pl.ds(pr, n // 2), :] = pltpu.bitcast(_ln(hf).astype(bf16), i32)

        def qkv_chunk(i, c):
            pr = _mo(i * PM, 8)
            lhs = ldb(ln1_s, pr, TM)
            c0 = c * CQ
            w = pltpu.bitcast(wqkv_p[:, pl.ds(c0, CQ)], bf16)
            r = jnp.dot(lhs, w, preferred_element_type=f32)
            r0 = _mo(i * TM + HALO, 8)
            for t in range(CQ // 128):
                tt = c0 // 128 + t
                piece = r[:, t * 128:(t + 1) * 128]
                if tt < NT:
                    piece = piece * (DH ** -0.5 * LOG2E)
                qkv_s[tt, pl.ds(r0, TM), :] = piece

        def qkv_pro(c, j):
            lhs = ldb(ln1_s, 0, TM, (j * KC, KC))
            w = pltpu.bitcast(wqkv_p[pl.ds(j * KC // 2, KC // 2), pl.ds(c * D, D)], bf16)
            r = jnp.dot(lhs, w, preferred_element_type=f32)
            for t in range(NT):
                tt = c * NT + t
                piece = r[:, t * 128:(t + 1) * 128]
                if c == 0:
                    piece = piece * (DH ** -0.5 * LOG2E)
                if j == 0:
                    qkv_s[tt, pl.ds(HALO, TM), :] = piece
                else:
                    qkv_s[tt, pl.ds(HALO, TM), :] += piece

        def attn_chunk(i, r):
            base = i * TM + HALO + r
            def ld(t, w):
                return qkv_s[t, pl.ds(base - DIL * w, R), :]
            xs = []
            for w in range(W):
                acc = None
                for t in range(NT):
                    p = qkv_s[t, pl.ds(_mo(base, 8), R), :] * ld(NT + t, w)
                    acc = p if acc is None else acc + p
                if not grp:
                    acc = acc + _lane_xor(acc, 1)
                    acc = acc + _lane_xor(acc, 2)
                xs.append(acc)
            if grp:
                xs = [a + _lane_xor(a, 1) for a in xs]
                xs = [a + _lane_xor(a, 2) for a in xs]
            for w in range(W):
                if r < DIL * w:
                    row = lax.broadcasted_iota(i32, (R, 128), 0) + (i * TM + r)
                    xs[w] = jnp.where(row >= DIL * w, xs[w], -1e9 * LOG2E)
            m = xs[0]
            for w in range(1, W):
                m = jnp.maximum(m, xs[w])
            ps = [jnp.exp2(x - m) for x in xs]
            ssum = ps[0]
            for w in range(1, W):
                ssum = ssum + ps[w]
            rcp = 1.0 / ssum
            for t in range(NT):
                acc = None
                for w in range(W):
                    p = ps[w] * ld(2 * NT + t, w)
                    acc = p if acc is None else acc + p
                o_s[pl.ds(r // 2, R // 2), pl.ds(t * 128, 128)] = pltpu.bitcast((acc * rcp).astype(bf16), i32)

        def wo_chunk(i, c):
            r0 = _mo((i + 1) * TM, 8); pr = _mo(i * PM, 8)
            c0 = c * CW_
            a = jnp.dot(pltpu.bitcast(o_s[...], bf16), pltpu.bitcast(wo_p[:, pl.ds(c0, CW_)], bf16), preferred_element_type=f32)
            h_s[pl.ds(r0, TM), pl.ds(c0, CW_)] = ldb(x_s, pr, TM, (c0, CW_)).astype(f32) + a

        def ffn_tile(row, TB, sem, mid=None):
            r0 = _mo(TM + row, 8); pr = _mo(PM + row // 2, 8); po = _mo(row // 2, 8)
            ln2 = ldb(ln2_s, pr, TB)
            acc = h_s[pl.ds(r0, TB), :]
            for j in range(F // FC):
                if mid is not None:
                    mid(j)
                a = jnp.dot(ln2, pltpu.bitcast(w1_s[:, pl.ds(j * FC, FC)], bf16), preferred_element_type=f32)
                a = jnp.maximum(a, 0.0).astype(bf16)
                acc = acc + jnp.dot(a, pltpu.bitcast(w2_s[pl.ds(j * FC // 2, FC // 2), :], bf16), preferred_element_type=f32)
            out_s[pl.ds(po, TB // 2), :] = pltpu.bitcast(acc.astype(bf16), i32)
            pltpu.make_async_copy(out_s.at[pl.ds(po, TB // 2), :], ob.at[pl.ds(po, TB // 2), :], out_sem.at[sem]).start()

        nattn = TM // R
        nln = TM // LNR
        def body_a(i, first=False):
            att = _split(nattn, NCH)
            lq = _split(nln, NCH)
            for c in range(NCH):
                if first and c == x2_wait_at:
                    cp_x2.wait()
                if first and c == wo_wait_at:
                    cp_wo.wait()
                    _permute_rows(wo_s, wo_p)
                for a in att[c]:
                    attn_chunk(i, a * R)
                if ln2_pos == "qkv" and not first:
                    for a in lq[c]:
                        ln2_rows(i - 1, a * LNR, LNR)
                if ln1_pos == "qkv":
                    for a in lq[c]:
                        ln1_rows(i + 2, a * LNR, LNR)
                qkv_chunk(i + 1, c)
            lw = _split(nln, NWO)
            for c in range(NWO):
                if ln2_pos == "wo" and not first:
                    for a in lw[c]:
                        ln2_rows(i - 1, a * LNR, LNR)
                if ln1_pos == "wo":
                    for a in lw[c]:
                        ln1_rows(i + 2, a * LNR, LNR)
                wo_chunk(i, c)

        with scope("pro"):
            cp_x0.start()
            for c in range(3):
                for j in range(KP):
                    cp_w[c][j].start()
            cp_x1.start(); cp_wo.start(); cp_x2.start(); cp_w1.start(); cp_w2.start()
            for t in range(NT, 3 * NT):
                qkv_s[t, pl.ds(0, HALO), :] = jnp.zeros((HALO, 128), f32)
            x_s[pl.ds(S // 2, PM), :] = jnp.zeros((PM, D), i32)
            cp_x0.wait()
            for a in range(nln):
                ln1_rows(0, a * LNR, LNR)
            seq = [(c, j) for c in range(3) for j in range(KP)]
            cp_w[0][0].wait()
            _permute_cols(wqkv_s, wqkv_p, 0, 0, KC // 2, PCH)
            for n, (c, j) in enumerate(seq):
                if n + 1 < len(seq):
                    c2, j2 = seq[n + 1]
                    cp_w[c2][j2].wait()
                    _permute_cols(wqkv_s, wqkv_p, c2 * D, j2 * KC // 2, KC // 2, PCH)
                else:
                    cp_x1.wait()
                    for a in range(nln):
                        ln1_rows(1, a * LNR, LNR)
                qkv_pro(c, j)
        with scope("phaseA"):
            body_a(0, first=True)
            def step(p, _):
                for u in range(unrollA):
                    body_a(1 + p * unrollA + u)
                return 0
            lax.fori_loop(0, (NA - 2) // unrollA, step, 0)
            for i in range(1 + ((NA - 2) // unrollA) * unrollA, NA - 1):
                body_a(i)
        with scope("trans"):
            i = NA - 1
            cp_w1.wait(); cp_w2.wait()
            for a in range(nln):
                ln2_rows(i - 1, a * LNR, LNR)
            nj = F // FC
            att = _split(nattn, wo_at)
            def mid(j):
                if j < wo_at:
                    for a in att[j]:
                        attn_chunk(i, a * R)
                if j == wo_at:
                    for c in range(NWO):
                        wo_chunk(i, c)
                    for a in range(nln):
                        ln2_rows(i, a * LNR, LNR)
            ffn_tile(0, T0, 0, mid)
        with scope("phaseB"):
            def fb(j, _):
                ffn_tile(T0 + j * TB, TB, 1 + j)
                return 0
            lax.fori_loop(0, NB, fb, 0)
        with scope("tail"):
            if TL:
                ffn_tile(T0 + NB * TB, TL, 1 + NB)
        pieces = [(0, T0)] + [(T0 + j * TB, TB) for j in range(NB)] + ([(T0 + NB * TB, TL)] if TL else [])
        for j, (rw, n) in enumerate(pieces):
            pltpu.make_async_copy(out_s.at[pl.ds(rw // 2, n // 2), :], ob.at[pl.ds(rw // 2, n // 2), :], out_sem.at[j]).wait()

    @jax.jit
    def f(A_x, A_wqkv, A_wo, B_x, B_w1, B_w2):
        x = A_x.reshape(S, D)
        anyspec = pl.BlockSpec(memory_space=pl.ANY)
        V = pltpu.VMEM
        out = pl.pallas_call(
            kernel,
            in_specs=[anyspec] * 5, out_specs=anyspec,
            out_shape=jax.ShapeDtypeStruct((S, D), bf16),
            scratch_shapes=[V((S // 2 + PM, D), i32), V((D // 2, 3 * D), i32), V((D // 2, 3 * D), i32), V((D // 2, D), i32), V((D // 2, D), i32),
                            V((D // 2, F), i32), V((F // 2, D), i32),
                            V((S // 2 + PM, D), i32), V((3 * NT, HALO + S, 128), f32),
                            V((TM // 2, D), i32), V((S + TM, D), f32), V((S // 2 + PM, D), i32), V((S // 2, D), i32),
                            pltpu.SemaphoreType.DMA((3 * KP + 6,)), pltpu.SemaphoreType.DMA((NB + 2,))],
            compiler_params=pltpu.CompilerParams(vmem_limit_bytes=120 * 2**20, flags=flags),
            name="v9",
        )(x, A_wqkv, A_wo, B_w1, B_w2)
        return out.reshape(1, S, D)
    return f


pallas_sequential_preLN__sliding_local_dilated__dense_activation_relu__prompt_kernel = make()
```

```python
import jax
import jax.numpy as jnp
from jax import lax
from jax.experimental import pallas as pl
from jax.experimental.pallas import tpu as pltpu

S, D, F = 2048, 1024, 3584
DH, W, DIL = 32, 8, 2
LANES = 128
NT = D // LANES
HALO = 16

TM = 256
NA = S // TM
PM = TM // 2
T0 = 128
TB = 320
NB = (S - T0) // TB
KC = 256
NK = D // KC
CQ = 256
FC = 512
R = 16
LNR = 32
WO_WAIT = 6
WO_AT = 5
assert T0 + NB * TB == S

LOG2E = 1.4426950408889634
QSCALE = DH ** -0.5 * LOG2E
NEG = -1e9 * LOG2E

f32, bf16, i32 = jnp.float32, jnp.bfloat16, jnp.int32


def _mo(x, m):
    return x if isinstance(x, int) else pl.multiple_of(x, m)


def _split(n, parts):
    b = [(n * j) // parts for j in range(parts + 1)]
    return [range(b[j], b[j + 1]) for j in range(parts)]


def _layernorm(xf):
    m = jnp.mean(xf, axis=-1, keepdims=True)
    c = xf - m
    v = jnp.mean(c * c, axis=-1, keepdims=True)
    return c * lax.rsqrt(v + 1e-5)


def _lane_xor(x, bit):
    idx = lax.broadcasted_iota(i32, x.shape, 1) ^ bit
    return jnp.take_along_axis(x, idx, axis=1)


def _permute_cols(src_ref, dst_ref, pr0, npr, c0):
    tiles = [src_ref[pl.ds(pr0, npr), pl.ds(c0 + t * LANES, LANES)] for t in range(NT)]
    lane = lax.broadcasted_iota(i32, (npr, LANES), 1)
    for tb, lb in ((4, 16), (2, 8), (1, 4)):
        hi = (lane & lb) != 0
        out = list(tiles)
        for t in range(NT):
            if t & tb:
                continue
            a, b = tiles[t], tiles[t | tb]
            s = _lane_xor(jnp.where(hi, a, b), lb)
            out[t] = jnp.where(hi, s, a)
            out[t | tb] = jnp.where(hi, b, s)
        tiles = out
    for t in range(NT):
        dst_ref[pl.ds(pr0, npr), pl.ds(c0 + t * LANES, LANES)] = tiles[t]


def _permute_rows(src_ref, dst_ref):
    cw = 512
    sub = lax.broadcasted_iota(i32, (8, cw), 0)
    m4 = (sub & 4) != 0
    m2 = (sub & 2) != 0
    for a in range(4):
        for h4 in range(2):
            for d4 in range(2):
                for c0 in range(0, D, cw):
                    v = {}
                    for h3 in range(2):
                        for h2 in range(2):
                            slab = (h4 << 5) | (h3 << 4) | (h2 << 3) | (a << 1) | d4
                            v[h3, h2] = src_ref[pl.ds(slab * 8, 8), pl.ds(c0, cw)]
                    for h2 in range(2):
                        x, y = v[0, h2], v[1, h2]
                        s = pltpu.roll(jnp.where(m4, x, y), 4, 0)
                        v[0, h2] = jnp.where(m4, s, x)
                        v[1, h2] = jnp.where(m4, y, s)
                    for h3 in range(2):
                        x, y = v[h3, 0], v[h3, 1]
                        v[h3, 0] = jnp.where(m2, pltpu.roll(y, 2, 0), x)
                        v[h3, 1] = jnp.where(m2, y, pltpu.roll(x, 6, 0))
                    for d3 in range(2):
                        for d2 in range(2):
                            slab = (d4 << 5) | (d3 << 4) | (d2 << 3) | (a << 1) | h4
                            dst_ref[pl.ds(slab * 8, 8), pl.ds(c0, cw)] = v[d3, d2]


def _kernel(x_hbm, wqkv_hbm, wo_hbm, w1_hbm, w2_hbm, out_hbm,
            x_s, wqkv_s, wqkv_p, wo_s, wo_p, w1_s, w2_s,
            ln1_s, qkv_s, o_s, h_s, ln2_s, out_s,
            w_sem, x_sem, out_sem):
    xb, wqb, wob, w1b, w2b, ob = (r.bitcast(i32) for r in
                                  (x_hbm, wqkv_hbm, wo_hbm, w1_hbm, w2_hbm, out_hbm))

    def cp_x(i):
        po = _mo(i * PM, 8)
        return pltpu.make_async_copy(xb.at[pl.ds(po, PM), :], x_s.at[pl.ds(po, PM), :], x_sem.at[i])

    def cp_wqkv(n):
        c, j = divmod(n, NK)
        idx = (pl.ds(j * KC // 2, KC // 2), pl.ds(c * D, D))
        return pltpu.make_async_copy(wqb.at[idx], wqkv_s.at[idx], w_sem.at[n])

    cp_wo = pltpu.make_async_copy(wob, wo_s, w_sem.at[3 * NK])
    cp_w1 = pltpu.make_async_copy(w1b, w1_s, w_sem.at[3 * NK + 1])
    cp_w2 = pltpu.make_async_copy(w2b, w2_s, w_sem.at[3 * NK + 2])

    def cp_out(row, n, sem):
        po = _mo(row // 2, 8)
        return pltpu.make_async_copy(out_s.at[pl.ds(po, n // 2), :], ob.at[pl.ds(po, n // 2), :],
                                     out_sem.at[sem])

    def ldb(ref, prow, nrows, c0=0, nc=None):
        nc = ref.shape[1] if nc is None else nc
        return pltpu.bitcast(ref[pl.ds(prow, nrows // 2), pl.ds(c0, nc)], bf16)

    def ln1_rows(i, a):
        pr = _mo(i * PM + a * (LNR // 2), 8)
        ln1_s[pl.ds(pr, LNR // 2), :] = pltpu.bitcast(
            _layernorm(ldb(x_s, pr, LNR).astype(f32)).astype(bf16), i32)

    def ln2_rows(i, a):
        r0 = _mo((i + 1) * TM + a * LNR, 8)
        pr = _mo((i + 1) * PM + a * (LNR // 2), 8)
        ln2_s[pl.ds(pr, LNR // 2), :] = pltpu.bitcast(
            _layernorm(h_s[pl.ds(r0, LNR), :]).astype(bf16), i32)

    def ln_tile(fn, i):
        for a in range(TM // LNR):
            fn(i, a)

    def qkv_chunk(i, c):
        lhs = ldb(ln1_s, _mo(i * PM, 8), TM)
        r = jnp.dot(lhs, ldb(wqkv_p, 0, D, c * CQ, CQ), preferred_element_type=f32)
        r0 = _mo(i * TM + HALO, 8)
        for t in range(CQ // LANES):
            tt = c * CQ // LANES + t
            piece = r[:, t * LANES:(t + 1) * LANES]
            qkv_s[tt, pl.ds(r0, TM), :] = piece * QSCALE if tt < NT else piece

    def qkv_first(n):
        c, j = divmod(n, NK)
        lhs = ldb(ln1_s, 0, TM, j * KC, KC)
        r = jnp.dot(lhs, ldb(wqkv_p, j * KC // 2, KC, c * D, D), preferred_element_type=f32)
        for t in range(NT):
            piece = r[:, t * LANES:(t + 1) * LANES]
            if c == 0:
                piece = piece * QSCALE
            if j == 0:
                qkv_s[c * NT + t, pl.ds(HALO, TM), :] = piece
            else:
                qkv_s[c * NT + t, pl.ds(HALO, TM), :] += piece

    def attn_chunk(i, r):
        base = i * TM + HALO + r

        def ld(t, w):
            return qkv_s[t, pl.ds(base - DIL * w, R), :]

        xs = []
        for w in range(W):
            acc = None
            for t in range(NT):
                p = qkv_s[t, pl.ds(_mo(base, 8), R), :] * ld(NT + t, w)
                acc = p if acc is None else acc + p
            xs.append((acc + _lane_xor(acc, 1)) + (_lane_xor(acc, 2) + _lane_xor(acc, 3)))
        for w in range(W):
            if r < DIL * w:
                row = lax.broadcasted_iota(i32, (R, LANES), 0) + (i * TM + r)
                xs[w] = jnp.where(row >= DIL * w, xs[w], NEG)
        m = xs[0]
        for w in range(1, W):
            m = jnp.maximum(m, xs[w])
        ps = [jnp.exp2(x - m) for x in xs]
        den = ps[0]
        for w in range(1, W):
            den = den + ps[w]
        rcp = 1.0 / den
        outs = [None] * NT
        for w in range(W):
            for t in range(NT):
                p = ps[w] * ld(2 * NT + t, w)
                outs[t] = p if outs[t] is None else outs[t] + p
        for t in range(NT):
            o_s[pl.ds(r // 2, R // 2), pl.ds(t * LANES, LANES)] = pltpu.bitcast(
                (outs[t] * rcp).astype(bf16), i32)

    def wo_chunk(i, c):
        a = jnp.dot(pltpu.bitcast(o_s[...], bf16), ldb(wo_p, 0, D, c * CQ, CQ),
                    preferred_element_type=f32)
        res = ldb(x_s, _mo(i * PM, 8), TM, c * CQ, CQ).astype(f32)
        h_s[pl.ds(_mo((i + 1) * TM, 8), TM), pl.ds(c * CQ, CQ)] = res + a

    def ffn_rows(row, n, sem, mid=None):
        ln2 = ldb(ln2_s, _mo(PM + row // 2, 8), n)
        acc = h_s[pl.ds(_mo(TM + row, 8), n), :]
        for j in range(F // FC):
            if mid is not None:
                mid(j)
            a = jnp.dot(ln2, ldb(w1_s, 0, D, j * FC, FC), preferred_element_type=f32)
            a = jnp.maximum(a, 0.0).astype(bf16)
            acc = acc + jnp.dot(a, ldb(w2_s, j * FC // 2, FC), preferred_element_type=f32)
        out_s[pl.ds(_mo(row // 2, 8), n // 2), :] = pltpu.bitcast(acc.astype(bf16), i32)
        cp_out(row, n, sem).start()

    nqkv, nwo, nattn, nln = 3 * D // CQ, D // CQ, TM // R, TM // LNR

    def tile_body(i, first=False):
        if first:
            att = [range(0)] * WO_WAIT + _split(nattn, nqkv - WO_WAIT)
        else:
            att = _split(nattn, nqkv)

            @pl.when(i + 2 < NA)
            def _():
                cp_x(i + 2).wait()
        for c in range(nqkv):
            if first and c == WO_WAIT:
                cp_wo.wait()
                cp_x(2).wait()
                _permute_rows(wo_s, wo_p)
            for a in att[c]:
                attn_chunk(i, a * R)
            qkv_chunk(i + 1, c)
        lw = _split(nln, nwo)
        for c in range(nwo):
            if not first:
                for a in lw[c]:
                    ln2_rows(i - 1, a)
            for a in lw[c]:
                ln1_rows(i + 2, a)
            wo_chunk(i, c)

    cp_x(0).start()
    for n in range(3 * NK):
        cp_wqkv(n).start()
    cp_x(1).start()
    cp_wo.start()
    for i in range(2, NA):
        cp_x(i).start()
    cp_w1.start()
    cp_w2.start()
    for t in range(NT, 3 * NT):
        qkv_s[t, pl.ds(0, HALO), :] = jnp.zeros((HALO, LANES), f32)
    x_s[pl.ds(S // 2, PM), :] = jnp.zeros((PM, D), i32)
    cp_x(0).wait()
    ln_tile(ln1_rows, 0)
    cp_wqkv(0).wait()
    _permute_cols(wqkv_s, wqkv_p, 0, KC // 2, 0)
    for n in range(3 * NK):
        if n + 1 < 3 * NK:
            c2, j2 = divmod(n + 1, NK)
            cp_wqkv(n + 1).wait()
            _permute_cols(wqkv_s, wqkv_p, j2 * KC // 2, KC // 2, c2 * D)
        else:
            cp_x(1).wait()
            ln_tile(ln1_rows, 1)
        qkv_first(n)

    tile_body(0, first=True)

    def a_step(p, carry):
        tile_body(1 + p)
        return carry
    lax.fori_loop(0, NA - 2, a_step, 0)

    last = NA - 1
    cp_w1.wait()
    cp_w2.wait()
    ln_tile(ln2_rows, last - 1)
    att_last = _split(nattn, WO_AT)

    def mid(j):
        if j < WO_AT:
            for a in att_last[j]:
                attn_chunk(last, a * R)
        if j == WO_AT:
            for c in range(nwo):
                wo_chunk(last, c)
            ln_tile(ln2_rows, last)
    ffn_rows(0, T0, 0, mid)

    def b_step(j, carry):
        ffn_rows(T0 + j * TB, TB, 1 + j)
        return carry
    lax.fori_loop(0, NB, b_step, 0)

    cp_out(0, T0, 0).wait()
    for j in range(NB):
        cp_out(T0 + j * TB, TB, 1 + j).wait()


@jax.jit
def pallas_sequential_preLN__sliding_local_dilated__dense_activation_relu__prompt_kernel(
    A_x: jax.Array,
    A_wqkv: jax.Array,
    A_wo: jax.Array,
    B_x: jax.Array,
    B_w1: jax.Array,
    B_w2: jax.Array,
):
    del B_x
    hbm = pl.BlockSpec(memory_space=pl.ANY)
    vmem = pltpu.VMEM
    out = pl.pallas_call(
        _kernel,
        in_specs=[hbm] * 5,
        out_specs=hbm,
        out_shape=jax.ShapeDtypeStruct((S, D), bf16),
        scratch_shapes=[
            vmem((S // 2 + PM, D), i32),
            vmem((D // 2, 3 * D), i32),
            vmem((D // 2, 3 * D), i32),
            vmem((D // 2, D), i32),
            vmem((D // 2, D), i32),
            vmem((D // 2, F), i32),
            vmem((F // 2, D), i32),
            vmem((S // 2 + PM, D), i32),
            vmem((3 * NT, HALO + S, LANES), f32),
            vmem((PM, D), i32),
            vmem((TM + S, D), f32),
            vmem((PM + S // 2, D), i32),
            vmem((S // 2, D), i32),
            pltpu.SemaphoreType.DMA((3 * NK + 3,)),
            pltpu.SemaphoreType.DMA((NA,)),
            pltpu.SemaphoreType.DMA((NB + 1,)),
        ],
        compiler_params=pltpu.CompilerParams(
            vmem_limit_bytes=120 * 2**20,
            flags={"XLA_TPU_EVENLY_DISTRIBUTE_CRITICAL_NODES": True},
        ),
    )(A_x.reshape(S, D), A_wqkv, A_wo, B_w1, B_w2)
    return out.reshape(1, S, D)
```

```python
import jax
import jax.numpy as jnp
from jax import lax
from jax.experimental import pallas as pl
from jax.experimental.pallas import tpu as pltpu

S, D, F = 2048, 1024, 3584
DH, W, DIL = 32, 8, 2
LANES = 128
NT = D // LANES
HALO = 16

TM = 256
NA = S // TM
PM = TM // 2
T0 = 128
TB = 320
NB = (S - T0) // TB
KC = 256
NK = D // KC
CQ = 256
FC = 512
R = 16
LNR = 32
WO_WAIT = 6
WO_AT = 5
assert T0 + NB * TB == S
AHEAD = 2
PF = 128

LOG2E = 1.4426950408889634
QSCALE = DH ** -0.5 * LOG2E
NEG = -1e9 * LOG2E

f32, bf16, i32 = jnp.float32, jnp.bfloat16, jnp.int32


def _mo(x, m):
    return x if isinstance(x, int) else pl.multiple_of(x, m)


def _split(n, parts):
    b = [(n * j) // parts for j in range(parts + 1)]
    return [range(b[j], b[j + 1]) for j in range(parts)]


def _layernorm(xf):
    m = jnp.mean(xf, axis=-1, keepdims=True)
    c = xf - m
    v = jnp.mean(c * c, axis=-1, keepdims=True)
    return c * lax.rsqrt(v + 1e-5)


def _lane_xor(x, bit):
    idx = lax.broadcasted_iota(i32, x.shape, 1) ^ bit
    return jnp.take_along_axis(x, idx, axis=1)


def _swap_tiles_lanes(tiles):
    lane = lax.broadcasted_iota(i32, tiles[0].shape, 1)
    for tb, lb in ((4, 16), (2, 8), (1, 4)):
        hi = (lane & lb) != 0
        out = list(tiles)
        for t in range(NT):
            if t & tb:
                continue
            a, b = tiles[t], tiles[t | tb]
            s = _lane_xor(jnp.where(hi, a, b), lb)
            out[t] = jnp.where(hi, s, a)
            out[t | tb] = jnp.where(hi, b, s)
        tiles = out
    return tiles


def _permute_cols(src_ref, dst_ref, pr0, npr, c0):
    tiles = [pltpu.bitcast(src_ref[pl.ds(2 * pr0, 2 * npr), pl.ds(c0 + t * LANES, LANES)], i32) for t in range(NT)]
    for t, v in enumerate(_swap_tiles_lanes(tiles)):
        dst_ref[pl.ds(pr0, npr), pl.ds(c0 + t * LANES, LANES)] = v


def _permute_rows(src_ref, dst_ref):
    cw = 512
    sub = lax.broadcasted_iota(i32, (8, cw), 0)
    m4 = (sub & 4) != 0
    m2 = (sub & 2) != 0
    for a in range(4):
        for h4 in range(2):
            for d4 in range(2):
                for c0 in range(0, D, cw):
                    v = {}
                    for h3 in range(2):
                        for h2 in range(2):
                            slab = (h4 << 5) | (h3 << 4) | (h2 << 3) | (a << 1) | d4
                            v[h3, h2] = pltpu.bitcast(src_ref[pl.ds(slab * 16, 16), pl.ds(c0, cw)], i32)
                    for h2 in range(2):
                        x, y = v[0, h2], v[1, h2]
                        s = pltpu.roll(jnp.where(m4, x, y), 4, 0)
                        v[0, h2] = jnp.where(m4, s, x)
                        v[1, h2] = jnp.where(m4, y, s)
                    for h3 in range(2):
                        x, y = v[h3, 0], v[h3, 1]
                        v[h3, 0] = jnp.where(m2, pltpu.roll(y, 2, 0), x)
                        v[h3, 1] = jnp.where(m2, y, pltpu.roll(x, 6, 0))
                    for d3 in range(2):
                        for d2 in range(2):
                            slab = (d4 << 5) | (d3 << 4) | (d2 << 3) | (a << 1) | h4
                            dst_ref[pl.ds(slab * 8, 8), pl.ds(c0, cw)] = v[d3, d2]


def _kernel(x_hbm, wqkv_hbm, wo_hbm, w1_hbm, w2_hbm, out_hbm,
            x_s, wqkv_s, wqkv_p, wo_s, wo_p, w1_s, w2_s,
            ln1_s, qkv_s, o_s, h_s, ln2_s, out_s,
            w_sem, x_sem, out_sem):
    def cp_x(i):
        po = _mo(i * TM, 16)
        return pltpu.make_async_copy(x_hbm.at[pl.ds(po, TM), :], x_s.at[pl.ds(po, TM), :], x_sem.at[i])

    def cp_wqkv(n):
        c, j = divmod(n, NK)
        idx = (pl.ds(j * KC, KC), pl.ds(c * D, D))
        return pltpu.make_async_copy(wqkv_hbm.at[idx], wqkv_s.at[idx], w_sem.at[n])

    cp_wo = pltpu.make_async_copy(wo_hbm, wo_s, w_sem.at[3 * NK])
    cp_w1 = pltpu.make_async_copy(w1_hbm, w1_s, w_sem.at[3 * NK + 1])
    cp_w2 = pltpu.make_async_copy(w2_hbm, w2_s, w_sem.at[3 * NK + 2])

    def cp_out(row, n, sem):
        po = _mo(row, 16)
        return pltpu.make_async_copy(out_s.at[pl.ds(po, n), :], out_hbm.at[pl.ds(po, n), :],
                                     out_sem.at[sem])

    def ldb(ref, prow, nrows, c0=0, nc=None):
        nc = ref.shape[1] if nc is None else nc
        if ref.dtype == bf16:
            return ref[pl.ds(_mo(2 * prow, 16), nrows), pl.ds(c0, nc)]
        return pltpu.bitcast(ref[pl.ds(prow, nrows // 2), pl.ds(c0, nc)], bf16)

    def ln1_rows(i, a):
        pr = _mo(i * PM + a * (LNR // 2), 8)
        ln1_s[pl.ds(pr, LNR // 2), :] = pltpu.bitcast(
            _layernorm(ldb(x_s, pr, LNR).astype(f32)).astype(bf16), i32)

    def ln2_rows(i, a):
        r0 = _mo((i + 1) * TM + a * LNR, 8)
        pr = _mo((i + 1) * PM + a * (LNR // 2), 8)
        ln2_s[pl.ds(pr, LNR // 2), :] = pltpu.bitcast(
            _layernorm(h_s[pl.ds(r0, LNR), :]).astype(bf16), i32)

    def ln_tile(fn, i):
        for a in range(TM // LNR):
            fn(i, a)

    def qkv_chunk(i, c):
        lhs = ldb(ln1_s, _mo(i * PM, 8), TM)
        r = jnp.dot(lhs, ldb(wqkv_p, 0, D, c * CQ, CQ), preferred_element_type=f32)
        r0 = _mo(i * TM + HALO, 8)
        for t in range(CQ // LANES):
            tt = c * CQ // LANES + t
            piece = r[:, t * LANES:(t + 1) * LANES]
            qkv_s[tt, pl.ds(r0, TM), :] = piece * QSCALE if tt < NT else piece

    def qkv_first(n):
        c, j = divmod(n, NK)
        lhs = ldb(ln1_s, 0, TM, j * KC, KC)
        r = jnp.dot(lhs, ldb(wqkv_s, j * KC // 2, KC, c * D, D), preferred_element_type=f32)
        for t in range(NT):
            piece = r[:, t * LANES:(t + 1) * LANES]
            if c == 0:
                piece = piece * QSCALE
            if j == 0:
                qkv_s[c * NT + t, pl.ds(HALO, TM), :] = piece
            else:
                qkv_s[c * NT + t, pl.ds(HALO, TM), :] += piece

    def permute_first(c, r0, n):
        tiles = [qkv_s[c * NT + t, pl.ds(HALO + r0, n), :] for t in range(NT)]
        for t, v in enumerate(_swap_tiles_lanes(tiles)):
            qkv_s[c * NT + t, pl.ds(HALO + r0, n), :] = v

    def attn_chunk(i, r):
        base = i * TM + HALO + r

        def ld(t, w):
            return qkv_s[t, pl.ds(base - DIL * w, R), :]

        xs = []
        for w in range(W):
            acc = None
            for t in range(NT):
                p = qkv_s[t, pl.ds(_mo(base, 8), R), :] * ld(NT + t, w)
                acc = p if acc is None else acc + p
            xs.append((acc + _lane_xor(acc, 1)) + (_lane_xor(acc, 2) + _lane_xor(acc, 3)))
        for w in range(W):
            if r < DIL * w:
                row = lax.broadcasted_iota(i32, (R, LANES), 0) + (i * TM + r)
                xs[w] = jnp.where(row >= DIL * w, xs[w], NEG)
        m = xs[0]
        for w in range(1, W):
            m = jnp.maximum(m, xs[w])
        ps = [jnp.exp2(x - m) for x in xs]
        den = ps[0]
        for w in range(1, W):
            den = den + ps[w]
        rcp = 1.0 / den
        outs = [None] * NT
        for w in range(W):
            for t in range(NT):
                p = ps[w] * ld(2 * NT + t, w)
                outs[t] = p if outs[t] is None else outs[t] + p
        for t in range(NT):
            o_s[pl.ds(r // 2, R // 2), pl.ds(t * LANES, LANES)] = pltpu.bitcast(
                (outs[t] * rcp).astype(bf16), i32)

    def wo_chunk(i, c):
        a = jnp.dot(pltpu.bitcast(o_s[...], bf16), ldb(wo_p, 0, D, c * CQ, CQ),
                    preferred_element_type=f32)
        res = ldb(x_s, _mo(i * PM, 8), TM, c * CQ, CQ).astype(f32)
        h_s[pl.ds(_mo((i + 1) * TM, 8), TM), pl.ds(c * CQ, CQ)] = res + a

    def ffn_rows(row, n, sem, mid=None):
        ln2 = ldb(ln2_s, _mo(PM + row // 2, 8), n)
        acc = h_s[pl.ds(_mo(TM + row, 8), n), :]
        for j in range(F // FC):
            if mid is not None:
                mid(j)
            a = jnp.dot(ln2, ldb(w1_s, 0, D, j * FC, FC), preferred_element_type=f32)
            a = jnp.maximum(a, 0.0).astype(bf16)
            acc = acc + jnp.dot(a, ldb(w2_s, j * FC // 2, FC), preferred_element_type=f32)
        out_s[pl.ds(_mo(row, 16), n), :] = acc.astype(bf16)
        cp_out(row, n, sem).start()

    nqkv, nwo, nattn, nln = 3 * D // CQ, D // CQ, TM // R, TM // LNR

    def tile_body(i, first=False):
        if first:
            att = [range(0)] * WO_WAIT + _split(nattn, nqkv - WO_WAIT)
        else:
            att = _split(nattn, nqkv)

            @pl.when(i + 2 < NA)
            def _():
                cp_x(i + 2).wait()
        for c in range(nqkv):
            if first and c == WO_WAIT:
                cp_wo.wait()
                cp_x(2).wait()
                _permute_rows(wo_s, wo_p)
            for a in att[c]:
                attn_chunk(i, a * R)
            qkv_chunk(i + 1, c)
        lw = _split(nln, nwo)
        for c in range(nwo):
            if not first:
                for a in lw[c]:
                    ln2_rows(i - 1, a)
            for a in lw[c]:
                ln1_rows(i + 2, a)
            wo_chunk(i, c)

    queue = [cp_x(0)] + [cp_wqkv(n) for n in range(3 * NK)] + [cp_x(1), cp_wo] + \
        [cp_x(i) for i in range(2, NA)] + [cp_w1, cp_w2]
    issued = [0]

    def issue(upto):
        while issued[0] < min(upto, len(queue)):
            queue[issued[0]].start()
            issued[0] += 1
    issue(1 + AHEAD)
    for t in range(NT, 3 * NT):
        qkv_s[t, pl.ds(0, HALO), :] = jnp.zeros((HALO, LANES), f32)
    x_s[pl.ds(S, TM), :] = jnp.zeros((TM, D), bf16)
    cp_x(0).wait()
    ln_tile(ln1_rows, 0)
    for n in range(3 * NK):
        c, j = divmod(n, NK)
        cp_wqkv(n).wait()
        issue(n + 2 + AHEAD if n + 1 < 3 * NK else len(queue))
        _permute_cols(wqkv_s, wqkv_p, j * KC // 2, KC // 2, c * D)
        qkv_first(n)
    cp_x(1).wait()
    ln_tile(ln1_rows, 1)
    for c in range(3):
        for r0 in range(0, TM, PF):
            permute_first(c, r0, PF)

    tile_body(0, first=True)

    def a_step(p, carry):
        tile_body(1 + p)
        return carry
    lax.fori_loop(0, NA - 2, a_step, 0)

    last = NA - 1
    cp_w1.wait()
    cp_w2.wait()
    ln_tile(ln2_rows, last - 1)
    att_last = _split(nattn, WO_AT)

    def mid(j):
        if j < WO_AT:
            for a in att_last[j]:
                attn_chunk(last, a * R)
        if j == WO_AT:
            for c in range(nwo):
                wo_chunk(last, c)
            ln_tile(ln2_rows, last)
    ffn_rows(0, T0, 0, mid)

    def b_step(j, carry):
        ffn_rows(T0 + j * TB, TB, 1 + j)
        return carry
    lax.fori_loop(0, NB, b_step, 0)

    cp_out(0, T0, 0).wait()
    for j in range(NB):
        cp_out(T0 + j * TB, TB, 1 + j).wait()


@jax.jit
def pallas_sequential_preLN__sliding_local_dilated__dense_activation_relu__prompt_kernel(
    A_x: jax.Array,
    A_wqkv: jax.Array,
    A_wo: jax.Array,
    B_x: jax.Array,
    B_w1: jax.Array,
    B_w2: jax.Array,
):
    del B_x
    hbm = pl.BlockSpec(memory_space=pl.ANY)
    vmem = pltpu.VMEM
    out = pl.pallas_call(
        _kernel,
        in_specs=[hbm] * 5,
        out_specs=hbm,
        out_shape=jax.ShapeDtypeStruct((S, D), bf16),
        scratch_shapes=[
            vmem((S + TM, D), bf16),
            vmem((D, 3 * D), bf16),
            vmem((D // 2, 3 * D), i32),
            vmem((D, D), bf16),
            vmem((D // 2, D), i32),
            vmem((D, F), bf16),
            vmem((F, D), bf16),
            vmem((S // 2 + PM, D), i32),
            vmem((3 * NT, HALO + S, LANES), f32),
            vmem((PM, D), i32),
            vmem((TM + S, D), f32),
            vmem((PM + S // 2, D), i32),
            vmem((S, D), bf16),
            pltpu.SemaphoreType.DMA((3 * NK + 3,)),
            pltpu.SemaphoreType.DMA((NA,)),
            pltpu.SemaphoreType.DMA((NB + 1,)),
        ],
        compiler_params=pltpu.CompilerParams(
            vmem_limit_bytes=120 * 2**20,
            flags={"XLA_TPU_EVENLY_DISTRIBUTE_CRITICAL_NODES": True},
        ),
    )(A_x.reshape(S, D), A_wqkv, A_wo, B_w1, B_w2)
    return out.reshape(1, S, D)
```
